```python
import jax
import jax.numpy as jnp

def _softmax(x, axis=-1):
    return jax.nn.softmax(x, axis=axis)

def _gelu(x):
    return jax.nn.gelu(x, approximate=True)

def _silu(x):
    return jax.nn.silu(x)

def _sigmoid(x):
    return jax.nn.sigmoid(x)

def _layernorm(x, axis=-1, eps=1e-05):
    m = jnp.mean(x, axis=axis, keepdims=True)
    v = jnp.var(x, axis=axis, keepdims=True)
    return (x - m) / jnp.sqrt(v + eps)

def _scatter_add(tgt, idx, src, axis=0):
    return tgt.at[idx].add(src)

def _segment_sum(src, seg, n):
    return jax.ops.segment_sum(src, seg, n)

class _Rng:

    def __init__(self, key):
        self._k = key

    def _next(self):
        self._k, sub = jax.random.split(self._k)
        return sub

    def normal(self, shape):
        return jax.random.normal(self._next(), shape, dtype=jnp.bfloat16)

    def randint(self, lo, hi, shape):
        return jax.random.randint(self._next(), shape, lo, hi, dtype=jnp.int32)

    def uniform(self, shape, lo=0.0, hi=1.0):
        return jax.random.uniform(self._next(), shape, jnp.bfloat16, lo, hi)

    def permutation(self, n):
        return jax.random.permutation(self._next(), n)
kernel_name = 'adaLN_cond__sliding_block_cached__glu_gated_glu__decode'

def setup_inputs():
    _rng = _Rng(jax.random.key(int.from_bytes(__import__("os").urandom(4), "little")))
    _w = lambda a: (lambda t: t.astype(jnp.bfloat16) if jnp.issubdtype(t.dtype, jnp.floating) else t)(jnp.asarray(a))

    def _A_setup():
        B, Sq, D = (8, 1, 512)
        Hq, Hkv, Sk, Dh = (32, 32, 4096, 128)
        assert Hq % Hkv == 0, (Hq, Hkv)
        return {'x': _w((lambda *s: _rng.normal(s) * 0.05)(B, Sq, D)), 'k_cache': _w((lambda *s: _rng.normal(s) * 0.05)(B, Hkv, Sk, Dh)), 'v_cache': _w((lambda *s: _rng.normal(s) * 0.05)(B, Hkv, Sk, Dh)), 'wq': _w((lambda *s: _rng.normal(s) * 0.05)(D, Hq * Dh) * D ** (-0.5)), 'wo': _w((lambda *s: _rng.normal(s) * 0.05)(Hq * Dh, D) * (Hq * Dh) ** (-0.5))}
    _A_in = _A_setup()

    def _B_setup():
        B, S, D, F = (8, 1, 512, 1376)
        return {'x': _w((lambda *s: _rng.normal(s) * 0.05)(B, S, D)), 'w_gate': _w((lambda *s: _rng.normal(s) * 0.05)(D, F)), 'w_up': _w((lambda *s: _rng.normal(s) * 0.05)(D, F)), 'w_down': _w((lambda *s: _rng.normal(s) * 0.05)(F, D))}
    _B_in = _B_setup()
    return {'A_x': _A_in['x'], 'A_k_cache': _A_in['k_cache'], 'A_v_cache': _A_in['v_cache'], 'A_wq': _A_in['wq'], 'A_wo': _A_in['wo'], 'B_x': _B_in['x'], 'B_w_gate': _B_in['w_gate'], 'B_w_up': _B_in['w_up'], 'B_w_down': _B_in['w_down'], 'c': _w((lambda *s: _rng.normal(s) * 0.05)(8, 512)), 'w_mod': _w((lambda *s: _rng.normal(s) * 0.05)(512, 6 * 512) * 512 ** (-0.5))}

def reference(A_x, A_k_cache, A_v_cache, A_wq, A_wo, B_x, B_w_gate, B_w_up, B_w_down, c, w_mod):

    def _A_ref(x, k_cache, v_cache, wq, wo):
        B, Sq, D = x.shape
        Hq, Dh = (32, 128)
        Hkv, Sk = (k_cache.shape[1], k_cache.shape[2])
        W = min(4096, max(256, Sk // 4))
        rep = Hq // Hkv
        q = (lambda x, *d: x.transpose(*d))((x @ wq).reshape(B, Sq, Hq, Dh), 0, 2, 1, 3)
        k = jnp.repeat(k_cache[:, :, Sk - W:, :], rep, axis=1)
        v = jnp.repeat(v_cache[:, :, Sk - W:, :], rep, axis=1)
        scores = jnp.einsum('bhqd,bhkd->bhqk', q, k) * Dh ** (-0.5)
        p = _softmax(scores, axis=-1)
        o = jnp.einsum('bhqk,bhkd->bhqd', p, v)
        return (lambda x, *d: x.transpose(*d))(o, 0, 2, 1, 3).reshape(B, Sq, Hq * Dh) @ wo

    def _B_ref(x, w_gate, w_up, w_down):
        g = jnp.einsum('bsd,df->bsf', x, w_gate)
        u = jnp.einsum('bsd,df->bsf', x, w_up)
        h = _sigmoid(g) * u
        return jnp.einsum('bsf,fd->bsd', h, w_down)
    x = A_x
    mod = (_silu(c) @ w_mod).reshape(c.shape[0], 6, 1, -1)
    sa, ca, ga, sb, cb, gb = (mod[:, 0].copy(), mod[:, 1].copy(), mod[:, 2].copy(), mod[:, 3].copy(), mod[:, 4].copy(), mod[:, 5].copy())
    h = _layernorm(x, axis=-1) * (1 + ca) + sa
    x = x + ga * _A_ref(h, A_k_cache, A_v_cache, A_wq, A_wo)
    h = _layernorm(x, axis=-1) * (1 + cb) + sb
    x = x + gb * _B_ref(h, B_w_gate, B_w_up, B_w_down)
    return x
```

```python
import jax
import jax.numpy as jnp
import jax.experimental.pallas as pl
import jax.experimental.pallas.tpu as pltpu
from jax import lax

B, D, H, DH, SK, F = 8, 512, 32, 128, 4096, 1376
W = min(4096, max(256, SK // 4))
EPS = 1e-5
NB = 3

_NT = (((1,), (1,)), ((), ()))


def _ln(x):
    m = jnp.mean(x, axis=-1, keepdims=True)
    d = x - m
    v = jnp.mean(d * d, axis=-1, keepdims=True)
    return d * lax.rsqrt(v + EPS)


def _kernel(x_hbm, k_hbm, v_hbm, wq_hbm, wo_hbm, wgt_hbm, wut_hbm, wd_hbm, c_hbm, wmod_hbm,
            o_ref,
            x_v, c_v, kbuf, vbuf, wq_v, wo_v, wgt_v, wut_v, wd_v, wmod_v, q_s, acc_s,
            sem_w, sem_k, sem_v):
    f32, bf16 = jnp.float32, jnp.bfloat16

    def k_copy(h, slot):
        return pltpu.make_async_copy(k_hbm.at[:, h, pl.ds(SK - W, W), :], kbuf.at[slot], sem_k.at[slot])

    def v_copy(h, slot):
        return pltpu.make_async_copy(v_hbm.at[:, h, pl.ds(SK - W, W), :], vbuf.at[slot], sem_v.at[slot])

    cp_x = pltpu.make_async_copy(x_hbm, x_v, sem_w.at[0])
    cp_c = pltpu.make_async_copy(c_hbm, c_v, sem_w.at[1])
    cp_wmod = pltpu.make_async_copy(wmod_hbm, wmod_v, sem_w.at[2])
    cp_wq = pltpu.make_async_copy(wq_hbm, wq_v, sem_w.at[3])
    cp_wo = pltpu.make_async_copy(wo_hbm, wo_v, sem_w.at[4])
    cp_wg = pltpu.make_async_copy(wgt_hbm, wgt_v, sem_w.at[5])
    cp_wu = pltpu.make_async_copy(wut_hbm, wut_v, sem_w.at[6])
    cp_wd = pltpu.make_async_copy(wd_hbm, wd_v, sem_w.at[7])

    cp_c.start()
    cp_x.start()
    cp_wmod.start()
    cp_wq.start()
    k_copy(0, 0).start()
    v_copy(0, 0).start()
    cp_wo.start()
    for s in range(1, NB):
        k_copy(s, s).start()
        v_copy(s, s).start()

    cp_c.wait()
    cp_wmod.wait()
    cc = c_v[...].astype(f32)
    sc = (cc * jax.nn.sigmoid(cc)).astype(bf16)
    mod = jnp.dot(sc, wmod_v[...], preferred_element_type=f32)
    sa, ca, ga, sb, cb, gb = [mod[:, i * D:(i + 1) * D] for i in range(6)]

    cp_x.wait()
    x = x_v[...].astype(f32)
    h1 = (_ln(x) * (1.0 + ca) + sa).astype(bf16)
    cp_wq.wait()
    q = jnp.dot(h1, wq_v[...], preferred_element_type=f32)
    for h in range(H):
        q_s[h] = q[:, h * DH:(h + 1) * DH]
    acc_s[...] = jnp.zeros((B, D), f32)
    cp_wo.wait()

    row_s = lax.broadcasted_iota(jnp.int32, (B, W), 0)
    row_o = lax.broadcasted_iota(jnp.int32, (B, DH), 0)
    scale = DH ** -0.5

    def head(h, carry):
        slot = lax.rem(h, NB)
        k_copy(h, slot).wait()
        qh = q_s[h].astype(bf16)
        s = None
        for b in range(B):
            sb_ = lax.dot_general(qh, kbuf[slot, b], _NT, preferred_element_type=f32)
            s = sb_ if b == 0 else jnp.where(row_s == b, sb_, s)

        @pl.when(h + NB < H)
        def _():
            k_copy(h + NB, slot).start()

        s = s * scale
        m = jnp.max(s, axis=-1, keepdims=True)
        e = jnp.exp(s - m)
        l = jnp.sum(e, axis=-1, keepdims=True)
        p = e.astype(bf16)
        v_copy(h, slot).wait()
        o = None
        for b in range(B):
            ob = jnp.dot(p, vbuf[slot, b], preferred_element_type=f32)
            o = ob if b == 0 else jnp.where(row_o == b, ob, o)

        @pl.when(h + NB < H)
        def _():
            v_copy(h + NB, slot).start()

        @pl.when(h == H - NB)
        def _():
            cp_wg.start()
            cp_wu.start()
            cp_wd.start()

        o = (o / l).astype(bf16)
        acc_s[...] += jnp.dot(o, wo_v[pl.ds(pl.multiple_of(h * DH, DH), DH), :],
                              preferred_element_type=f32)
        return carry

    lax.fori_loop(0, H, head, 0)

    x1 = x + ga * acc_s[...]
    h2 = (_ln(x1) * (1.0 + cb) + sb).astype(bf16)
    cp_wg.wait()
    g = lax.dot_general(h2, wgt_v[...], _NT, preferred_element_type=f32)
    cp_wu.wait()
    u = lax.dot_general(h2, wut_v[...], _NT, preferred_element_type=f32)
    hh = (jax.nn.sigmoid(g) * u).astype(bf16)
    cp_wd.wait()
    y = jnp.dot(hh, wd_v[...], preferred_element_type=f32)
    o_ref[...] = (x1 + gb * y).astype(o_ref.dtype)


@jax.jit
def pallas_adaLN_cond__sliding_block_cached__glu_gated_glu__decode_kernel(
    A_x: jax.Array,
    A_k_cache: jax.Array,
    A_v_cache: jax.Array,
    A_wq: jax.Array,
    A_wo: jax.Array,
    B_x: jax.Array,
    B_w_gate: jax.Array,
    B_w_up: jax.Array,
    B_w_down: jax.Array,
    c: jax.Array,
    w_mod: jax.Array,
):
    del B_x
    bf16, f32 = jnp.bfloat16, jnp.float32
    hbm = pl.BlockSpec(memory_space=pltpu.HBM)
    out = pl.pallas_call(
        _kernel,
        in_specs=[hbm] * 10,
        out_specs=pl.BlockSpec(memory_space=pltpu.VMEM),
        out_shape=jax.ShapeDtypeStruct((B, D), A_x.dtype),
        scratch_shapes=[
            pltpu.VMEM((B, D), bf16),
            pltpu.VMEM((B, D), bf16),
            pltpu.VMEM((NB, B, W, DH), bf16),
            pltpu.VMEM((NB, B, W, DH), bf16),
            pltpu.VMEM((D, H * DH), bf16),
            pltpu.VMEM((H * DH, D), bf16),
            pltpu.VMEM((F, D), bf16),
            pltpu.VMEM((F, D), bf16),
            pltpu.VMEM((F, D), bf16),
            pltpu.VMEM((D, 6 * D), bf16),
            pltpu.VMEM((H, B, DH), f32),
            pltpu.VMEM((B, D), f32),
            pltpu.SemaphoreType.DMA((8,)),
            pltpu.SemaphoreType.DMA((NB,)),
            pltpu.SemaphoreType.DMA((NB,)),
        ],
        compiler_params=pltpu.CompilerParams(vmem_limit_bytes=64 * 1024 * 1024),
    )(A_x.reshape(B, D), A_k_cache, A_v_cache, A_wq, A_wo,
      B_w_gate.T, B_w_up.T, B_w_down, c, w_mod)
    return out.reshape(B, 1, D)
```

```python
import jax
import jax.numpy as jnp
import jax.experimental.pallas as pl
import jax.experimental.pallas.tpu as pltpu
from jax import lax

B, D, H, DH, SK, F = 8, 512, 32, 128, 4096, 1376
W = min(4096, max(256, SK // 4))
EPS = 1e-5

NB = 3
NS = NB + 1
R = 64
E, ER = 2, 128
FS = F - E * ER
LAST = 256

_NT = (((1,), (1,)), ((), ()))


def _layernorm(x):
    m = jnp.mean(x, axis=-1, keepdims=True)
    d = x - m
    v = jnp.mean(d * d, axis=-1, keepdims=True)
    return d * lax.rsqrt(v + EPS)


def _kernel(x_hbm, k_hbm, v_hbm, wq_hbm, wo_hbm, wgt_hbm, wut_hbm, wd_hbm, c_hbm, wmod_hbm,
            o_hbm,
            x_v, c_v, kbuf, vbuf, wq_v, wo_v, wgt_v, wut_v, wd_v, wmod_v, q_s, acc_s, o_v,
            v_sm, wd_sm, ring, side, misc):
    f32, bf16 = jnp.float32, jnp.bfloat16
    w0 = SK - W

    def k_copy(h):
        return pltpu.make_async_copy(k_hbm.at[:, h, pl.ds(w0, W), :], kbuf.at[h % NB], ring.at[h % NB])

    def v_copy(h):
        return pltpu.make_async_copy(v_hbm.at[:, h, pl.ds(w0, W - R), :],
                                     vbuf.at[h % NB, :, pl.ds(0, W - R), :], ring.at[h % NB])

    def v_hop1(h):
        return pltpu.make_async_copy(v_hbm.at[:, h, pl.ds(SK - R, R), :], v_sm.at[h % NS], side.at[h % NS])

    def v_hop2(h):
        return pltpu.make_async_copy(v_sm.at[h % NS], vbuf.at[h % NB, :, pl.ds(W - R, R), :], ring.at[h % NB])

    def wd_hop1(i):
        return pltpu.make_async_copy(wd_hbm.at[pl.ds(FS + i * ER, ER), :], wd_sm.at[i], side.at[(H + i) % NS])

    def wd_hop2(i):
        return pltpu.make_async_copy(wd_sm.at[i], wd_v.at[pl.ds(FS + i * ER, ER), :], side.at[(H + i) % NS])

    prologue = [pltpu.make_async_copy(s, d, misc.at[0]) for s, d in (
        (c_hbm, c_v), (x_hbm, x_v), (wmod_hbm, wmod_v), (wq_hbm, wq_v), (wo_hbm, wo_v))]
    gate_up = [pltpu.make_async_copy(s, d, misc.at[0]) for s, d in ((wgt_hbm, wgt_v), (wut_hbm, wut_v))]
    wd_main = pltpu.make_async_copy(wd_hbm.at[LAST:FS, :], wd_v.at[LAST:FS, :], ring.at[(H - 2) % NB])
    wd_last = pltpu.make_async_copy(wd_hbm.at[0:LAST, :], wd_v.at[0:LAST, :], ring.at[(H - 1) % NB])
    out_copy = pltpu.make_async_copy(o_v, o_hbm, misc.at[0])

    for cp in prologue:
        cp.start()
    for g in range(NS):
        v_hop1(g).start()
    for g in range(NB):
        v_hop1(g).wait()
        k_copy(g).start()
        v_copy(g).start()
        v_hop2(g).start()

    for cp in prologue:
        cp.wait()
    cc = c_v[...].astype(f32)
    mod = jnp.dot((cc * jax.nn.sigmoid(cc)).astype(bf16), wmod_v[...], preferred_element_type=f32)
    sa, ca, ga, sb, cb, gb = [mod[:, i * D:(i + 1) * D] for i in range(6)]
    x = x_v[...].astype(f32)
    h1 = (_layernorm(x) * (1.0 + ca) + sa).astype(bf16)
    q = jnp.dot(h1, wq_v[...], preferred_element_type=f32)
    for h in range(H):
        q_s[h] = q[:, h * DH:(h + 1) * DH]
    acc_s[...] = jnp.zeros((B, D), f32)

    row_s = lax.broadcasted_iota(jnp.int32, (B, W), 0)
    row_o = lax.broadcasted_iota(jnp.int32, (B, DH), 0)

    def head(h, carry):
        slot = h % NB
        k_copy(h).wait()
        v_copy(h).wait()
        v_hop2(h).wait()

        @pl.when(h + NS < H)
        def _():
            v_hop1(h + NS).start()

        for i in range(E):
            @pl.when(h + NS == H + i)
            def _():
                wd_hop1(i).start()

        qh = q_s[h].astype(bf16)
        s = None
        for b in range(B):
            sb_ = lax.dot_general(qh, kbuf[slot, b], _NT, preferred_element_type=f32)
            s = sb_ if b == 0 else jnp.where(row_s == b, sb_, s)

        @pl.when(h + NB < H)
        def _():
            k_copy(h + NB).start()

        s = s * DH ** -0.5
        e = jnp.exp(s - jnp.max(s, axis=-1, keepdims=True))
        denom = jnp.sum(e, axis=-1, keepdims=True)
        p = e.astype(bf16)
        o = None
        for b in range(B):
            ob = jnp.dot(p, vbuf[slot, b], preferred_element_type=f32)
            o = ob if b == 0 else jnp.where(row_o == b, ob, o)

        @pl.when(h + NB < H)
        def _():
            v_copy(h + NB).start()
            v_hop1(h + NB).wait()
            v_hop2(h + NB).start()

        for i in range(E):
            @pl.when(h + NB == H + i)
            def _():
                wd_hop1(i).wait()
                wd_hop2(i).start()

        @pl.when(h == H - 3)
        def _():
            for cp in gate_up:
                cp.start()

        @pl.when(h == H - 2)
        def _():
            wd_main.start()

        @pl.when(h == H - 1)
        def _():
            wd_last.start()

        o = (o / denom).astype(bf16)
        acc_s[...] += jnp.dot(o, wo_v[pl.ds(pl.multiple_of(h * DH, DH), DH), :],
                              preferred_element_type=f32)
        return carry

    lax.fori_loop(0, H, head, 0)

    x1 = x + ga * acc_s[...]
    h2 = (_layernorm(x1) * (1.0 + cb) + sb).astype(bf16)
    for cp in gate_up:
        cp.wait()
    g = lax.dot_general(h2, wgt_v[...], _NT, preferred_element_type=f32)
    u = lax.dot_general(h2, wut_v[...], _NT, preferred_element_type=f32)
    hid = (jax.nn.sigmoid(g) * u).astype(bf16)
    wd_main.wait()
    for i in range(E):
        wd_hop2(i).wait()
    acc_s[...] = x1 + gb * jnp.dot(hid[:, LAST:F], wd_v[LAST:F, :], preferred_element_type=f32)
    wd_last.wait()
    y = jnp.dot(hid[:, 0:LAST], wd_v[0:LAST, :], preferred_element_type=f32)
    o_v[...] = (acc_s[...] + gb * y).astype(o_v.dtype)
    out_copy.start()
    out_copy.wait()


@jax.jit
def pallas_adaLN_cond__sliding_block_cached__glu_gated_glu__decode_kernel(
    A_x: jax.Array,
    A_k_cache: jax.Array,
    A_v_cache: jax.Array,
    A_wq: jax.Array,
    A_wo: jax.Array,
    B_x: jax.Array,
    B_w_gate: jax.Array,
    B_w_up: jax.Array,
    B_w_down: jax.Array,
    c: jax.Array,
    w_mod: jax.Array,
):
    del B_x
    bf16, f32 = jnp.bfloat16, jnp.float32
    hbm = pl.BlockSpec(memory_space=pltpu.HBM)
    out = pl.pallas_call(
        _kernel,
        in_specs=[hbm] * 10,
        out_specs=hbm,
        out_shape=jax.ShapeDtypeStruct((B, D), A_x.dtype),
        scratch_shapes=[
            pltpu.VMEM((B, D), bf16),
            pltpu.VMEM((B, D), bf16),
            pltpu.VMEM((NB, B, W, DH), bf16),
            pltpu.VMEM((NB, B, W, DH), bf16),
            pltpu.VMEM((D, H * DH), bf16),
            pltpu.VMEM((H * DH, D), bf16),
            pltpu.VMEM((F, D), bf16),
            pltpu.VMEM((F, D), bf16),
            pltpu.VMEM((F, D), bf16),
            pltpu.VMEM((D, 6 * D), bf16),
            pltpu.VMEM((H, B, DH), f32),
            pltpu.VMEM((B, D), f32),
            pltpu.VMEM((B, D), bf16),
            pltpu.SMEM((NS, B, R, DH), bf16),
            pltpu.SMEM((E, ER, D), bf16),
            pltpu.SemaphoreType.DMA((NB,)),
            pltpu.SemaphoreType.DMA((NS,)),
            pltpu.SemaphoreType.DMA((1,)),
        ],
        compiler_params=pltpu.CompilerParams(vmem_limit_bytes=64 * 1024 * 1024),
    )(A_x.reshape(B, D), A_k_cache, A_v_cache, A_wq, A_wo,
      B_w_gate.T, B_w_up.T, B_w_down, c, w_mod)
    return out.reshape(B, 1, D)
```

```python
import jax
import jax.numpy as jnp
import jax.experimental.pallas as pl
import jax.experimental.pallas.tpu as pltpu
from jax import lax

B, D, H, DH, SK, F = 8, 512, 32, 128, 4096, 1376
W = min(4096, max(256, SK // 4))
EPS = 1e-5

NB = 3
NS = NB + 1
R = 64
LK, LV = 240, 128
E, ER = 2, 128
FS = F - E * ER
LAST = 256
NSLAB = 8

_NT = (((1,), (1,)), ((), ()))


def _layernorm(x):
    m = jnp.mean(x, axis=-1, keepdims=True)
    d = x - m
    v = jnp.mean(d * d, axis=-1, keepdims=True)
    return d * lax.rsqrt(v + EPS)


def _kernel(x_hbm, k_hbm, v_hbm, wq_hbm, wo_hbm, wgt_hbm, wut_hbm, wd_hbm, c_hbm, wmod_hbm,
            o_hbm,
            x_v, c_v, kbuf, vbuf, wq_v, wo_v, wgt_v, wut_v, wd_v, wmod_v, q_s, acc_s, o_v,
            k_sm, wd_sm, ring, side, misc):
    f32, bf16 = jnp.float32, jnp.bfloat16
    w0 = SK - W
    msem = misc.at[0]

    def wait_filled(buf, sem):
        pltpu.make_async_copy(buf, buf, sem).wait()

    def start_window(hbm, buf, h, rows, piece):
        def body(j, carry):
            a = pl.multiple_of(j * piece, 8)
            pltpu.make_async_copy(hbm.at[:, h, pl.ds(w0 + a, piece), :],
                                  buf.at[h % NB, :, pl.ds(a, piece), :], ring.at[h % NB]).start()
            return carry
        lax.fori_loop(0, rows // piece, body, 0)

    def start_k(h):
        start_window(k_hbm, kbuf, h, W - R, LK)

    def start_v(h):
        start_window(v_hbm, vbuf, h, W, LV)

    def start_slabs(src, dst, rows, cols):
        def body(j, carry):
            a = pl.ds(pl.multiple_of(j * rows, 8), rows)
            for c0 in range(0, src.shape[2], cols):
                pltpu.make_async_copy(src.at[:, a, c0:c0 + cols], dst.at[:, a, c0:c0 + cols], msem).start()
            return carry
        lax.fori_loop(0, src.shape[1] // rows, body, 0)

    def k_hop1(h):
        return pltpu.make_async_copy(k_hbm.at[:, h, pl.ds(SK - R, R), :], k_sm.at[h % NS], side.at[h % NS])

    def k_hop2(h):
        return pltpu.make_async_copy(k_sm.at[h % NS], kbuf.at[h % NB, :, pl.ds(W - R, R), :], ring.at[h % NB])

    def wd_hop1(i):
        return pltpu.make_async_copy(wd_hbm.at[pl.ds(FS + i * ER, ER), :], wd_sm.at[i], side.at[(H + i) % NS])

    def wd_hop2(i):
        return pltpu.make_async_copy(wd_sm.at[i], wd_v.at[pl.ds(FS + i * ER, ER), :], side.at[(H + i) % NS])

    wd_main = pltpu.make_async_copy(wd_hbm.at[LAST:FS, :], wd_v.at[LAST:FS, :], ring.at[(H - 2) % NB])
    wd_last = pltpu.make_async_copy(wd_hbm.at[0:LAST, :], wd_v.at[0:LAST, :], ring.at[(H - 1) % NB])

    pltpu.make_async_copy(c_hbm, c_v, msem).start()
    pltpu.make_async_copy(x_hbm, x_v, msem).start()
    for g in range(NS):
        k_hop1(g).start()
    start_slabs(wmod_hbm, wmod_v, 8, 6 * D)
    start_slabs(wq_hbm, wq_v, 8, H * DH // 2)
    start_slabs(wo_hbm, wo_v, 32, D)
    for g in range(NB):
        k_hop1(g).wait()
        start_k(g)
        start_v(g)
        k_hop2(g).start()

    for buf in (c_v, x_v, wmod_v, wq_v, wo_v):
        wait_filled(buf, msem)
    cc = c_v[...].astype(f32)
    mod = jnp.dot((cc * jax.nn.sigmoid(cc)).astype(bf16), wmod_v[...].reshape(D, 6 * D),
                  preferred_element_type=f32)
    sa, ca, ga, sb, cb, gb = [mod[:, i * D:(i + 1) * D] for i in range(6)]
    x = x_v[...].astype(f32)
    h1 = (_layernorm(x) * (1.0 + ca) + sa).astype(bf16)
    q = jnp.dot(h1, wq_v[...].reshape(D, H * DH), preferred_element_type=f32)
    for h in range(H):
        q_s[h] = q[:, h * DH:(h + 1) * DH]
    acc_s[...] = jnp.zeros((B, D), f32)

    row_s = lax.broadcasted_iota(jnp.int32, (B, W), 0)
    row_o = lax.broadcasted_iota(jnp.int32, (B, DH), 0)
    wo_heads = wo_v.reshape(H, DH, D)

    def head(h, carry):
        slot = h % NB
        wait_filled(kbuf.at[slot], ring.at[slot])
        wait_filled(vbuf.at[slot], ring.at[slot])

        @pl.when(h + NS < H)
        def _():
            k_hop1(h + NS).start()

        for i in range(E):
            @pl.when(h + NS == H + i)
            def _():
                wd_hop1(i).start()

        qh = q_s[h].astype(bf16)
        s = None
        for b in range(B):
            sb_ = lax.dot_general(qh, kbuf[slot, b], _NT, preferred_element_type=f32)
            s = sb_ if b == 0 else jnp.where(row_s == b, sb_, s)

        @pl.when(h + NB < H)
        def _():
            start_k(h + NB)

        s = s * DH ** -0.5
        e = jnp.exp(s - jnp.max(s, axis=-1, keepdims=True))
        denom = jnp.sum(e, axis=-1, keepdims=True)
        p = e.astype(bf16)
        o = None
        for b in range(B):
            ob = jnp.dot(p, vbuf[slot, b], preferred_element_type=f32)
            o = ob if b == 0 else jnp.where(row_o == b, ob, o)

        @pl.when(h + NB < H)
        def _():
            start_v(h + NB)
            k_hop1(h + NB).wait()
            k_hop2(h + NB).start()

        for i in range(E):
            @pl.when(h + NB == H + i)
            def _():
                wd_hop1(i).wait()
                wd_hop2(i).start()

        @pl.when(h == H - 3)
        def _():
            pltpu.make_async_copy(wgt_hbm, wgt_v, msem).start()
            pltpu.make_async_copy(wut_hbm, wut_v, msem).start()

        @pl.when(h == H - 2)
        def _():
            wd_main.start()

        @pl.when(h == H - 1)
        def _():
            wd_last.start()

        o = (o / denom).astype(bf16)
        acc_s[...] += jnp.dot(o, wo_heads[h], preferred_element_type=f32)
        return carry

    lax.fori_loop(0, H, head, 0)

    x1 = x + ga * acc_s[...]
    h2 = (_layernorm(x1) * (1.0 + cb) + sb).astype(bf16)
    wait_filled(wgt_v, msem)
    wait_filled(wut_v, msem)
    g = lax.dot_general(h2, wgt_v[...], _NT, preferred_element_type=f32)
    u = lax.dot_general(h2, wut_v[...], _NT, preferred_element_type=f32)
    hid = (jax.nn.sigmoid(g) * u).astype(bf16)
    wd_main.wait()
    for i in range(E):
        wd_hop2(i).wait()
    acc_s[...] = x1 + gb * jnp.dot(hid[:, LAST:F], wd_v[LAST:F, :], preferred_element_type=f32)
    wd_last.wait()
    y = jnp.dot(hid[:, 0:LAST], wd_v[0:LAST, :], preferred_element_type=f32)
    o_v[...] = (acc_s[...] + gb * y).astype(o_v.dtype)
    out_copy = pltpu.make_async_copy(o_v, o_hbm, msem)
    out_copy.start()
    out_copy.wait()


@jax.jit
def pallas_adaLN_cond__sliding_block_cached__glu_gated_glu__decode_kernel(
    A_x: jax.Array,
    A_k_cache: jax.Array,
    A_v_cache: jax.Array,
    A_wq: jax.Array,
    A_wo: jax.Array,
    B_x: jax.Array,
    B_w_gate: jax.Array,
    B_w_up: jax.Array,
    B_w_down: jax.Array,
    c: jax.Array,
    w_mod: jax.Array,
):
    del B_x
    bf16, f32 = jnp.bfloat16, jnp.float32
    hbm = pl.BlockSpec(memory_space=pltpu.HBM)
    wmod_shape = (NSLAB, D // NSLAB, 6 * D)
    wq_shape = (NSLAB, D // NSLAB, H * DH)
    wo_shape = (NSLAB, H * DH // NSLAB, D)
    out = pl.pallas_call(
        _kernel,
        in_specs=[hbm] * 10,
        out_specs=hbm,
        out_shape=jax.ShapeDtypeStruct((B, D), A_x.dtype),
        scratch_shapes=[
            pltpu.VMEM((B, D), bf16),
            pltpu.VMEM((B, D), bf16),
            pltpu.VMEM((NB, B, W, DH), bf16),
            pltpu.VMEM((NB, B, W, DH), bf16),
            pltpu.VMEM(wq_shape, bf16),
            pltpu.VMEM(wo_shape, bf16),
            pltpu.VMEM((F, D), bf16),
            pltpu.VMEM((F, D), bf16),
            pltpu.VMEM((F, D), bf16),
            pltpu.VMEM(wmod_shape, bf16),
            pltpu.VMEM((H, B, DH), f32),
            pltpu.VMEM((B, D), f32),
            pltpu.VMEM((B, D), bf16),
            pltpu.SMEM((NS, B, R, DH), bf16),
            pltpu.SMEM((E, ER, D), bf16),
            pltpu.SemaphoreType.DMA((NB,)),
            pltpu.SemaphoreType.DMA((NS,)),
            pltpu.SemaphoreType.DMA((1,)),
        ],
        compiler_params=pltpu.CompilerParams(vmem_limit_bytes=64 * 1024 * 1024),
    )(A_x.reshape(B, D), A_k_cache, A_v_cache, A_wq.reshape(wq_shape), A_wo.reshape(wo_shape),
      B_w_gate.T, B_w_up.T, B_w_down, c, w_mod.reshape(wmod_shape))
    return out.reshape(B, 1, D)
```

```python
import jax
import jax.numpy as jnp
import jax.experimental.pallas as pl
import jax.experimental.pallas.tpu as pltpu
from jax import lax

B, D, H, DH, SK, F = 8, 512, 32, 128, 4096, 1376
W = min(4096, max(256, SK // 4))
EPS = 1e-5

NB = 3
NS = NB + 1
R = 64
LK, LV = 240, 128
E, ER = 2, 144
FS = F - E * ER
LAST = 256
NSLAB = 8

_NT = (((1,), (1,)), ((), ()))


def _layernorm(x):
    m = jnp.mean(x, axis=-1, keepdims=True)
    d = x - m
    v = jnp.mean(d * d, axis=-1, keepdims=True)
    return d * lax.rsqrt(v + EPS)


def _kernel(x_hbm, k_hbm, v_hbm, wq_hbm, wo_hbm, wgt_hbm, wut_hbm, wd_hbm, c_hbm, wmod_hbm,
            o_hbm,
            x_v, c_v, kbuf, vbuf, wq_v, wo_v, wgt_v, wut_v, wd_v, wmod_v, q_s, acc_s, o_v,
            k_sm, wd_sm, ring, side, misc):
    f32, bf16 = jnp.float32, jnp.bfloat16
    w0 = SK - W
    msem = misc.at[0]

    def wait_filled(buf, sem):
        pltpu.make_async_copy(buf, buf, sem).wait()

    def start_window(hbm, buf, h, rows, piece):
        def body(j, carry):
            a = pl.multiple_of(j * piece, 8)
            pltpu.make_async_copy(hbm.at[:, h, pl.ds(w0 + a, piece), :],
                                  buf.at[h % NB, :, pl.ds(a, piece), :], ring.at[h % NB]).start()
            return carry
        lax.fori_loop(0, rows // piece, body, 0)

    def start_k(h):
        start_window(k_hbm, kbuf, h, W - R, LK)

    def start_v(h):
        start_window(v_hbm, vbuf, h, W, LV)

    def start_slabs(src, dst, rows, cols):
        def body(j, carry):
            a = pl.ds(pl.multiple_of(j * rows, 8), rows)
            for c0 in range(0, src.shape[2], cols):
                pltpu.make_async_copy(src.at[:, a, c0:c0 + cols], dst.at[:, a, c0:c0 + cols], msem).start()
            return carry
        lax.fori_loop(0, src.shape[1] // rows, body, 0)

    def k_hop1(h):
        return pltpu.make_async_copy(k_hbm.at[:, h, pl.ds(SK - R, R), :], k_sm.at[h % NS], side.at[h % 2])

    def k_hop2(h):
        return pltpu.make_async_copy(k_sm.at[h % NS], kbuf.at[h % NB, :, pl.ds(W - R, R), :], ring.at[h % NB])

    def wd_hop1(i):
        return pltpu.make_async_copy(wd_hbm.at[pl.ds(FS + i * ER, ER), :], wd_sm.at[i], side.at[(H + i) % 2])

    def wd_hop2(i):
        return pltpu.make_async_copy(wd_sm.at[i], wd_v.at[pl.ds(FS + i * ER, ER), :], side.at[(H + i) % 2])

    wd_main = pltpu.make_async_copy(wd_hbm.at[LAST:FS, :], wd_v.at[LAST:FS, :], ring.at[(H - 2) % NB])
    wd_last = pltpu.make_async_copy(wd_hbm.at[0:LAST, :], wd_v.at[0:LAST, :], ring.at[(H - 1) % NB])

    pltpu.make_async_copy(c_hbm, c_v, msem).start()
    pltpu.make_async_copy(x_hbm, x_v, msem).start()
    k_hop1(0).start()
    k_hop1(1).start()
    start_slabs(wmod_hbm, wmod_v, 8, 3 * D)
    start_slabs(wq_hbm, wq_v, 8, H * DH // 4)
    start_slabs(wo_hbm, wo_v, 16, D)
    for g in range(NB):
        k_hop1(g).wait()
        if g + 2 < NS:
            k_hop1(g + 2).start()
        start_k(g)
        start_v(g)
        k_hop2(g).start()

    for buf in (c_v, x_v, wmod_v, wq_v, wo_v):
        wait_filled(buf, msem)
    cc = c_v[...].astype(f32)
    mod = jnp.dot((cc * jax.nn.sigmoid(cc)).astype(bf16), wmod_v[...].reshape(D, 6 * D),
                  preferred_element_type=f32)
    sa, ca, ga, sb, cb, gb = [mod[:, i * D:(i + 1) * D] for i in range(6)]
    x = x_v[...].astype(f32)
    h1 = (_layernorm(x) * (1.0 + ca) + sa).astype(bf16)
    q = jnp.dot(h1, wq_v[...].reshape(D, H * DH), preferred_element_type=f32)
    for h in range(H):
        q_s[h] = q[:, h * DH:(h + 1) * DH]
    acc_s[...] = jnp.zeros((B, D), f32)

    row_s = lax.broadcasted_iota(jnp.int32, (B, W), 0)
    row_o = lax.broadcasted_iota(jnp.int32, (B, DH), 0)
    wo_heads = wo_v.reshape(H, DH, D)

    def head(h, carry):
        slot = h % NB
        wait_filled(kbuf.at[slot], ring.at[slot])
        wait_filled(vbuf.at[slot], ring.at[slot])

        @pl.when(h + NS < H)
        def _():
            k_hop1(h + NS).start()

        for i in range(E):
            @pl.when(h + NS == H + i)
            def _():
                wd_hop1(i).start()

        qh = q_s[h].astype(bf16)
        s = None
        for b in range(B):
            sb_ = lax.dot_general(qh, kbuf[slot, b], _NT, preferred_element_type=f32)
            s = sb_ if b == 0 else jnp.where(row_s == b, sb_, s)

        @pl.when(h + NB < H)
        def _():
            start_k(h + NB)

        s = s * DH ** -0.5
        e = jnp.exp(s - jnp.max(s, axis=-1, keepdims=True))
        denom = jnp.sum(e, axis=-1, keepdims=True)
        p = e.astype(bf16)
        o = None
        for b in range(B):
            ob = jnp.dot(p, vbuf[slot, b], preferred_element_type=f32)
            o = ob if b == 0 else jnp.where(row_o == b, ob, o)

        @pl.when(h + NB < H)
        def _():
            start_v(h + NB)
            k_hop1(h + NB).wait()
            k_hop2(h + NB).start()

        for i in range(E):
            @pl.when(h + NB == H + i)
            def _():
                wd_hop1(i).wait()
                wd_hop2(i).start()

        @pl.when(h == H - 3)
        def _():
            pltpu.make_async_copy(wgt_hbm, wgt_v, msem).start()
            pltpu.make_async_copy(wut_hbm, wut_v, msem).start()

        @pl.when(h == H - 2)
        def _():
            wd_main.start()

        @pl.when(h == H - 1)
        def _():
            wd_last.start()

        o = (o / denom).astype(bf16)
        acc_s[...] += jnp.dot(o, wo_heads[h], preferred_element_type=f32)
        return carry

    lax.fori_loop(0, H, head, 0)

    x1 = x + ga * acc_s[...]
    h2 = (_layernorm(x1) * (1.0 + cb) + sb).astype(bf16)
    wait_filled(wgt_v, msem)
    wait_filled(wut_v, msem)
    g = lax.dot_general(h2, wgt_v[...], _NT, preferred_element_type=f32)
    u = lax.dot_general(h2, wut_v[...], _NT, preferred_element_type=f32)
    hid = (jax.nn.sigmoid(g) * u).astype(bf16)
    wd_main.wait()
    for i in range(E):
        wd_hop2(i).wait()
    acc_s[...] = x1 + gb * jnp.dot(hid[:, LAST:F], wd_v[LAST:F, :], preferred_element_type=f32)
    wd_last.wait()
    y = jnp.dot(hid[:, 0:LAST], wd_v[0:LAST, :], preferred_element_type=f32)
    o_v[...] = (acc_s[...] + gb * y).astype(o_v.dtype)
    out_copy = pltpu.make_async_copy(o_v, o_hbm, msem)
    out_copy.start()
    out_copy.wait()


@jax.jit
def pallas_adaLN_cond__sliding_block_cached__glu_gated_glu__decode_kernel(
    A_x: jax.Array,
    A_k_cache: jax.Array,
    A_v_cache: jax.Array,
    A_wq: jax.Array,
    A_wo: jax.Array,
    B_x: jax.Array,
    B_w_gate: jax.Array,
    B_w_up: jax.Array,
    B_w_down: jax.Array,
    c: jax.Array,
    w_mod: jax.Array,
):
    del B_x
    bf16, f32 = jnp.bfloat16, jnp.float32
    hbm = pl.BlockSpec(memory_space=pltpu.HBM)
    wmod_shape = (NSLAB, D // NSLAB, 6 * D)
    wq_shape = (NSLAB, D // NSLAB, H * DH)
    wo_shape = (NSLAB, H * DH // NSLAB, D)
    out = pl.pallas_call(
        _kernel,
        in_specs=[hbm] * 10,
        out_specs=hbm,
        out_shape=jax.ShapeDtypeStruct((B, D), A_x.dtype),
        scratch_shapes=[
            pltpu.VMEM((B, D), bf16),
            pltpu.VMEM((B, D), bf16),
            pltpu.VMEM((NB, B, W, DH), bf16),
            pltpu.VMEM((NB, B, W, DH), bf16),
            pltpu.VMEM(wq_shape, bf16),
            pltpu.VMEM(wo_shape, bf16),
            pltpu.VMEM((F, D), bf16),
            pltpu.VMEM((F, D), bf16),
            pltpu.VMEM((F, D), bf16),
            pltpu.VMEM(wmod_shape, bf16),
            pltpu.VMEM((H, B, DH), f32),
            pltpu.VMEM((B, D), f32),
            pltpu.VMEM((B, D), bf16),
            pltpu.SMEM((NS, B, R, DH), bf16),
            pltpu.SMEM((E, ER, D), bf16),
            pltpu.SemaphoreType.DMA((NB,)),
            pltpu.SemaphoreType.DMA((2,)),
            pltpu.SemaphoreType.DMA((1,)),
        ],
        compiler_params=pltpu.CompilerParams(vmem_limit_bytes=64 * 1024 * 1024),
    )(A_x.reshape(B, D), A_k_cache, A_v_cache, A_wq.reshape(wq_shape), A_wo.reshape(wo_shape),
      B_w_gate.T, B_w_up.T, B_w_down, c, w_mod.reshape(wmod_shape))
    return out.reshape(B, 1, D)
```
